```python
import jax
import jax.numpy as jnp

def _softmax(x, axis=-1):
    return jax.nn.softmax(x, axis=axis)

def _gelu(x):
    return jax.nn.gelu(x, approximate=True)

def _silu(x):
    return jax.nn.silu(x)

def _sigmoid(x):
    return jax.nn.sigmoid(x)

def _layernorm(x, axis=-1, eps=1e-05):
    m = jnp.mean(x, axis=axis, keepdims=True)
    v = jnp.var(x, axis=axis, keepdims=True)
    return (x - m) / jnp.sqrt(v + eps)

def _scatter_add(tgt, idx, src, axis=0):
    return tgt.at[idx].add(src)

def _segment_sum(src, seg, n):
    return jax.ops.segment_sum(src, seg, n)

class _Rng:

    def __init__(self, key):
        self._k = key

    def _next(self):
        self._k, sub = jax.random.split(self._k)
        return sub

    def normal(self, shape):
        return jax.random.normal(self._next(), shape, dtype=jnp.bfloat16)

    def randint(self, lo, hi, shape):
        return jax.random.randint(self._next(), shape, lo, hi, dtype=jnp.int32)

    def uniform(self, shape, lo=0.0, hi=1.0):
        return jax.random.uniform(self._next(), shape, jnp.bfloat16, lo, hi)

    def permutation(self, n):
        return jax.random.permutation(self._next(), n)
kernel_name = 'adaLN_cond__sliding_block_cached__glu_gated_bilinear__decode'

def setup_inputs():
    _rng = _Rng(jax.random.key(int.from_bytes(__import__("os").urandom(4), "little")))
    _w = lambda a: (lambda t: t.astype(jnp.bfloat16) if jnp.issubdtype(t.dtype, jnp.floating) else t)(jnp.asarray(a))

    def _A_setup():
        B, Sq, D = (1, 1, 640)
        Hq, Hkv, Sk, Dh = (32, 32, 32768, 192)
        assert Hq % Hkv == 0, (Hq, Hkv)
        return {'x': _w((lambda *s: _rng.normal(s) * 0.05)(B, Sq, D)), 'k_cache': _w((lambda *s: _rng.normal(s) * 0.05)(B, Hkv, Sk, Dh)), 'v_cache': _w((lambda *s: _rng.normal(s) * 0.05)(B, Hkv, Sk, Dh)), 'wq': _w((lambda *s: _rng.normal(s) * 0.05)(D, Hq * Dh) * D ** (-0.5)), 'wo': _w((lambda *s: _rng.normal(s) * 0.05)(Hq * Dh, D) * (Hq * Dh) ** (-0.5))}
    _A_in = _A_setup()

    def _B_setup():
        B, S, D, F = (1, 1, 640, 1536)
        return {'x': _w((lambda *s: _rng.normal(s) * 0.05)(B, S, D)), 'w_gate': _w((lambda *s: _rng.normal(s) * 0.05)(D, F) * D ** (-0.5)), 'w_up': _w((lambda *s: _rng.normal(s) * 0.05)(D, F) * D ** (-0.5)), 'w_down': _w((lambda *s: _rng.normal(s) * 0.05)(F, D) * F ** (-0.5))}
    _B_in = _B_setup()
    return {'A_x': _A_in['x'], 'A_k_cache': _A_in['k_cache'], 'A_v_cache': _A_in['v_cache'], 'A_wq': _A_in['wq'], 'A_wo': _A_in['wo'], 'B_x': _B_in['x'], 'B_w_gate': _B_in['w_gate'], 'B_w_up': _B_in['w_up'], 'B_w_down': _B_in['w_down'], 'c': _w((lambda *s: _rng.normal(s) * 0.05)(1, 640)), 'w_mod': _w((lambda *s: _rng.normal(s) * 0.05)(640, 6 * 640) * 640 ** (-0.5))}

def reference(A_x, A_k_cache, A_v_cache, A_wq, A_wo, B_x, B_w_gate, B_w_up, B_w_down, c, w_mod):

    def _A_ref(x, k_cache, v_cache, wq, wo):
        B, Sq, D = x.shape
        Hq, Dh = (32, 192)
        Hkv, Sk = (k_cache.shape[1], k_cache.shape[2])
        W = min(4096, max(256, Sk // 4))
        rep = Hq // Hkv
        q = (lambda x, *d: x.transpose(*d))((x @ wq).reshape(B, Sq, Hq, Dh), 0, 2, 1, 3)
        k = jnp.repeat(k_cache[:, :, Sk - W:, :], rep, axis=1)
        v = jnp.repeat(v_cache[:, :, Sk - W:, :], rep, axis=1)
        scores = jnp.einsum('bhqd,bhkd->bhqk', q, k) * Dh ** (-0.5)
        p = _softmax(scores, axis=-1)
        o = jnp.einsum('bhqk,bhkd->bhqd', p, v)
        return (lambda x, *d: x.transpose(*d))(o, 0, 2, 1, 3).reshape(B, Sq, Hq * Dh) @ wo

    def _B_ref(x, w_gate, w_up, w_down):
        g = jnp.einsum('bsd,df->bsf', x, w_gate)
        u = jnp.einsum('bsd,df->bsf', x, w_up)
        h = g * u
        return jnp.einsum('bsf,fd->bsd', h, w_down)
    x = A_x
    mod = (_silu(c) @ w_mod).reshape(c.shape[0], 6, 1, -1)
    sa, ca, ga, sb, cb, gb = (mod[:, 0].copy(), mod[:, 1].copy(), mod[:, 2].copy(), mod[:, 3].copy(), mod[:, 4].copy(), mod[:, 5].copy())
    h = _layernorm(x, axis=-1) * (1 + ca) + sa
    x = x + ga * _A_ref(h, A_k_cache, A_v_cache, A_wq, A_wo)
    h = _layernorm(x, axis=-1) * (1 + cb) + sb
    x = x + gb * _B_ref(h, B_w_gate, B_w_up, B_w_down)
    return x
```

```python
import functools

import jax
import jax.numpy as jnp
import numpy as np
from jax import lax
import jax.experimental.pallas as pl
import jax.experimental.pallas.tpu as pltpu

F32 = jnp.float32
BF16 = jnp.bfloat16

_HQ = 32
_DH = 192
_EPS = 1e-5

_NBUF = 3
_CW = 256
_FC = 256


def _rbf(v):
    return v.astype(BF16).astype(F32)


def _layernorm_rows(v):
    m = jnp.mean(v, axis=-1, keepdims=True)
    d = v - m
    var = jnp.mean(d * d, axis=-1, keepdims=True)
    return d * lax.rsqrt(var + _EPS)


def _kernel(x_hbm, c_hbm, kt_hbm, vt_hbm, wq_hbm, wo_hbm, wg_hbm, wu_hbm, wd_hbm, wm_hbm,
            out_ref,
            xbuf, cbuf, kbuf, vbuf, wq, wo, wg, wu, wd, wm, q_scr, p_scr,
            sem_w, sem_d, sem_k, sem_v,
            *, D, FF, SK, W):
    H, DH, NB = _HQ, _DH, _NBUF
    c0 = SK - W
    n_dc = FF // _FC
    scale = float(np.asarray(DH ** -0.5, dtype=BF16))

    def k_copy(h, slot):
        return pltpu.make_async_copy(
            kt_hbm.at[pl.ds(h * DH, DH), pl.ds(c0, W)], kbuf.at[slot], sem_k.at[slot])

    def v_copy(h, slot):
        return pltpu.make_async_copy(
            vt_hbm.at[pl.ds(h * DH, DH), pl.ds(c0, W)], vbuf.at[slot], sem_v.at[slot])

    cp_x = pltpu.make_async_copy(x_hbm, xbuf, sem_w.at[0])
    cp_c = pltpu.make_async_copy(c_hbm, cbuf, sem_w.at[1])
    cp_wm = pltpu.make_async_copy(wm_hbm, wm, sem_w.at[2])
    cp_wq = pltpu.make_async_copy(wq_hbm, wq, sem_w.at[3])
    cp_wo = pltpu.make_async_copy(wo_hbm, wo, sem_w.at[4])
    cp_wg = pltpu.make_async_copy(wg_hbm, wg, sem_w.at[5])
    cp_wu = pltpu.make_async_copy(wu_hbm, wu, sem_w.at[6])
    cp_wd = [pltpu.make_async_copy(wd_hbm.at[pl.ds(j * _FC, _FC), :],
                                   wd.at[pl.ds(j * _FC, _FC), :], sem_d.at[j])
             for j in range(n_dc)]

    cp_c.start()
    cp_x.start()
    cp_wm.start()
    cp_wq.start()
    cp_wo.start()
    for h in range(NB):
        k_copy(h, h).start()
        v_copy(h, h).start()
    cp_wg.start(priority=1)
    cp_wu.start(priority=1)
    for cp in cp_wd:
        cp.start(priority=1)

    cp_c.wait()
    cp_x.wait()
    c = cbuf[...].astype(F32)
    sc = c * (1.0 / (1.0 + jnp.exp(-c)))
    sc8 = jnp.broadcast_to(sc, (8, D)).astype(BF16)
    x = jnp.broadcast_to(xbuf[...].astype(F32), (8, D))
    cp_wm.wait()
    mod = _rbf(jnp.dot(sc8, wm[...], preferred_element_type=F32))
    sa, ca, ga = mod[:, 0:D], mod[:, D:2 * D], mod[:, 2 * D:3 * D]
    sb, cb, gb = mod[:, 3 * D:4 * D], mod[:, 4 * D:5 * D], mod[:, 5 * D:6 * D]
    h1 = (_rbf(_layernorm_rows(x)) * _rbf(1.0 + ca) + sa).astype(BF16)
    cp_wq.wait()
    q = jnp.dot(h1, wq[...], preferred_element_type=F32)
    for h in range(H):
        q_scr[h] = q[:, h * DH:(h + 1) * DH]
    cp_wo.wait()

    def head_body(h, attn):
        slot = lax.rem(h, NB)
        k_copy(h, slot).wait()
        qh = q_scr[h].astype(BF16)
        s = jnp.dot(qh, kbuf[slot], preferred_element_type=F32)
        s = _rbf(_rbf(s) * scale)

        @pl.when(h + NB < H)
        def _():
            k_copy(h + NB, slot).start()

        m = jnp.max(s, axis=-1, keepdims=True)
        e = jnp.exp(s - m)
        l = jnp.sum(e, axis=-1, keepdims=True)
        p_scr[...] = _rbf(e * (1.0 / l))

        v_copy(h, slot).wait()

        def pv_body(j, acc):
            off = pl.multiple_of(j * _CW, _CW)
            vt = vbuf[slot, :, pl.ds(off, _CW)].astype(F32)
            pj = p_scr[:, pl.ds(off, _CW)]
            prod = vt.reshape(DH // 8, 8, _CW) * pj[None]
            for t in range(_CW // 128):
                acc = acc + prod[:, :, t * 128:(t + 1) * 128]
            return acc

        acc = lax.fori_loop(0, W // _CW, pv_body, jnp.zeros((DH // 8, 8, 128), F32))

        @pl.when(h + NB < H)
        def _():
            v_copy(h + NB, slot).start()

        o = _rbf(jnp.sum(acc, axis=-1, keepdims=True))
        row0 = pl.multiple_of(h * DH, 64)
        woh = wo[pl.ds(row0, DH), :].astype(F32).reshape(DH // 8, 8, D)
        return attn + jnp.sum(woh * o, axis=0)

    attn8 = lax.fori_loop(0, H, head_body, jnp.zeros((8, D), F32))
    attn = _rbf(jnp.sum(attn8, axis=0, keepdims=True))

    x1 = _rbf(x + _rbf(ga * attn))
    h2 = (_rbf(_layernorm_rows(x1)) * _rbf(1.0 + cb) + sb).astype(BF16)
    cp_wg.wait()
    g = _rbf(jnp.dot(h2, wg[...], preferred_element_type=F32))
    cp_wu.wait()
    u = _rbf(jnp.dot(h2, wu[...], preferred_element_type=F32))
    hh = (g * u).astype(BF16)
    y = jnp.zeros((8, D), F32)
    for j in range(n_dc):
        cp_wd[j].wait()
        y = y + jnp.dot(hh[:, j * _FC:(j + 1) * _FC], wd[pl.ds(j * _FC, _FC), :],
                        preferred_element_type=F32)
    x2 = x1 + _rbf(gb * _rbf(y))
    out_ref[...] = x2[0:1, :].astype(out_ref.dtype)


@jax.jit
def pallas_adaLN_cond__sliding_block_cached__glu_gated_bilinear__decode_kernel(
    A_x: jax.Array,
    A_k_cache: jax.Array,
    A_v_cache: jax.Array,
    A_wq: jax.Array,
    A_wo: jax.Array,
    B_x: jax.Array,
    B_w_gate: jax.Array,
    B_w_up: jax.Array,
    B_w_down: jax.Array,
    c: jax.Array,
    w_mod: jax.Array,
):
    B, SQ, D = A_x.shape
    _, HKV, SK, DH = A_k_cache.shape
    assert B == 1 and SQ == 1 and HKV == _HQ and DH == _DH
    W = min(4096, max(256, SK // 4))
    FF = B_w_gate.shape[1]

    kt = jnp.swapaxes(A_k_cache, 2, 3).reshape(HKV * DH, SK)
    vt = jnp.swapaxes(A_v_cache, 2, 3).reshape(HKV * DH, SK)
    x2d = A_x.reshape(1, D)

    any_spec = pl.BlockSpec(memory_space=pl.ANY)
    out = pl.pallas_call(
        functools.partial(_kernel, D=D, FF=FF, SK=SK, W=W),
        out_shape=jax.ShapeDtypeStruct((1, D), A_x.dtype),
        in_specs=[any_spec] * 10,
        out_specs=pl.BlockSpec(memory_space=pltpu.VMEM),
        scratch_shapes=[
            pltpu.VMEM((1, D), BF16),
            pltpu.VMEM((1, D), BF16),
            pltpu.VMEM((_NBUF, DH, W), BF16),
            pltpu.VMEM((_NBUF, DH, W), BF16),
            pltpu.VMEM(A_wq.shape, BF16),
            pltpu.VMEM(A_wo.shape, BF16),
            pltpu.VMEM(B_w_gate.shape, BF16),
            pltpu.VMEM(B_w_up.shape, BF16),
            pltpu.VMEM(B_w_down.shape, BF16),
            pltpu.VMEM(w_mod.shape, BF16),
            pltpu.VMEM((_HQ, 8, DH), F32),
            pltpu.VMEM((8, W), F32),
            pltpu.SemaphoreType.DMA((7,)),
            pltpu.SemaphoreType.DMA((FF // _FC,)),
            pltpu.SemaphoreType.DMA((_NBUF,)),
            pltpu.SemaphoreType.DMA((_NBUF,)),
        ],
        compiler_params=pltpu.CompilerParams(vmem_limit_bytes=96 * 1024 * 1024),
    )(x2d, c, kt, vt, A_wq, A_wo, B_w_gate, B_w_up, B_w_down, w_mod)
    return out.reshape(B, SQ, D)
```

```python
import functools

import jax
import jax.numpy as jnp
import numpy as np
from jax import lax
import jax.experimental.pallas as pl
import jax.experimental.pallas.tpu as pltpu

F32 = jnp.float32
BF16 = jnp.bfloat16

_HQ = 32
_DH = 192
_EPS = 1e-5

_CW = 128
_TPG = 8
_NG = 4
_NS = 4
_BG, _FG = 1, 0


def _rbf(v):
    return v.astype(BF16).astype(F32)


def _layernorm_rows(v):
    m = jnp.mean(v, axis=-1, keepdims=True)
    d = v - m
    var = jnp.mean(d * d, axis=-1, keepdims=True)
    return d * lax.rsqrt(var + _EPS)


def _dot(a, b):
    return jnp.dot(a, b, preferred_element_type=F32)


def _kernel(x_hbm, c_hbm, kt_hbm, vt_hbm, wq_hbm, wo_hbm, wg_hbm, wu_hbm, wd_hbm, wm_hbm,
            out_ref,
            xbuf, cbuf, kbuf, vbuf, wq, wo, wg, wu, wd, wm, q_scr, h_scr, p_scr,
            sem, sem_x,
            *, D, FF, SK, W):
    H, DH = _HQ, _DH
    GW = _CW * _TPG
    NP = H // 2
    NPOS = 4 * _NG
    LA = _NS - 1
    RB = D // NP
    c0 = SK - W
    scale = float(np.asarray(DH ** -0.5, dtype=BF16))
    cp = pltpu.make_async_copy

    def mul(v, k):
        return v * k if isinstance(v, int) else pl.multiple_of(v * k, 8)

    def bg_copy(m, g, i):
        src, dst = (kt_hbm, kbuf) if (g % 8) < _NG else (vt_hbm, vbuf)
        j = g % _NG
        row = mul(m, 2 * DH) + (g // 8) * DH
        return cp(src.at[pl.ds(row, DH), pl.ds(c0 + j * GW + i * _CW, _CW)],
                  dst.at[j, :, pl.ds(i * _CW, _CW)], sem.at[g % _NS])

    def wo_piece(hh, k):
        return lambda m, s: cp(wo_hbm.at[pl.ds(mul(m, 2 * DH) + hh * DH + 8 * k, 8), :],
                               wo.at[hh, pl.ds(8 * k, 8), :], s)

    def wq_piece(k):
        return lambda m, s: cp(
            wq_hbm.at[pl.ds(16 * k, 16), pl.ds(pl.multiple_of((m + 1) * 2 * DH, 128), 2 * DH)],
            wq.at[pl.ds(16 * k, 16), :], s)

    def blk_piece(src, dst, k, col0, ncols, shift):
        r, cc = divmod(k, (src.shape[1] - col0) // ncols)

        def f(m, s):
            row = mul(m + shift, RB) + 8 * r
            idx = (pl.ds(row, 8), pl.ds(col0 + cc * ncols, ncols))
            return cp(src.at[idx], dst.at[idx], s)
        return f

    def wd_piece(r0, n):
        return lambda m, s: cp(wd_hbm.at[pl.ds(r0, n), :], wd.at[pl.ds(r0, n), :], s)

    n_h = FF // 2
    late = ([blk_piece(wg_hbm, wg, k, 0, n_h, 0) for k in range(10)]
            + [blk_piece(wu_hbm, wu, k, 0, n_h, 0) for k in range(6)]
            + [blk_piece(wu_hbm, wu, k, 0, n_h, 1) for k in range(6, 10)]
            + [blk_piece(wm_hbm, wm, k, 2 * D, D, 1) for k in range(20)])
    flat = ([wo_piece(0, k) for k in range(24)] + [wq_piece(k) for k in range(40)]
            + [wo_piece(1, k) for k in range(24)] + late)
    assert len(flat) == NPOS * _TPG
    fg_mid = [flat[g * _TPG:(g + 1) * _TPG] for g in range(NPOS)]
    fg_last = list(fg_mid)
    for n, g in enumerate((3, 4, 5, 6, 7, 13, 14, 15)):
        fg_last[g] = [wd_piece(8 * (n * _TPG + i), 8) for i in range(_TPG)]
    wd_early = 8 * 8 * _TPG
    wd_tail = [(wd_early, 512), (wd_early + 512, 384), (wd_early + 896, 128)]
    assert wd_tail[-1][0] + wd_tail[-1][1] == FF
    tail_cp = [wd_piece(r0, n)(0, sem.at[(NPOS + t) % _NS]) for t, (r0, n) in enumerate(wd_tail)]

    cp_c = cp(c_hbm, cbuf, sem_x.at[0])
    cp_x = cp(x_hbm, xbuf, sem_x.at[0])
    cp_wma = cp(wm_hbm.at[:, pl.ds(0, 2 * D)], wm.at[:, pl.ds(0, 2 * D)], sem_x.at[0])
    cp_wq0 = cp(wq_hbm.at[:, pl.ds(0, 2 * DH)], wq, sem.at[LA])

    cp_c.start(priority=_FG)
    cp_x.start(priority=_FG)
    cp_wma.start(priority=_BG)
    cp_wq0.start(priority=_BG)
    for g in range(LA):
        for i in range(_TPG):
            bg_copy(0, g, i).start(priority=_BG)
            fg_mid[NPOS - LA + g][i](-1, sem.at[g]).start(priority=_FG)

    cp_c.wait()
    cp_x.wait()
    cp_wma.wait()
    c = cbuf[...].astype(F32)
    sc = c * (1.0 / (1.0 + jnp.exp(-c)))
    sc8 = jnp.broadcast_to(sc, (8, D)).astype(BF16)
    x = jnp.broadcast_to(xbuf[...].astype(F32), (8, D))
    mod_a = _rbf(_dot(sc8, wm[:, 0:2 * D]))
    sa, ca = mod_a[:, 0:D], mod_a[:, D:2 * D]
    h_scr[...] = _rbf(_rbf(_layernorm_rows(x)) * _rbf(1.0 + ca)) + sa

    def project_q():
        q2 = _dot(h_scr[...].astype(BF16), wq[...])
        q_scr[0] = q2[:, 0:DH]
        q_scr[1] = q2[:, DH:2 * DH]

    cp_wq0.wait()
    project_q()

    def pair_body(m, attn8, last):
        fg = fg_last if last else fg_mid
        mods = []
        s_parts, acc = [], None
        for g in range(NPOS):
            pm, pfg = (m - 1, fg_mid) if g < LA else (m, fg)
            for i in range(_TPG):
                pfg[(g - LA) % NPOS][i](pm, sem.at[g % _NS]).wait()
            for i in range(_TPG):
                bg_copy(m, g, i).wait()
                gn = g + LA
                if gn < NPOS:
                    bg_copy(m, gn, i).start(priority=_BG)
                elif not last:
                    bg_copy(m + 1, gn - NPOS, i).start(priority=_BG)
                elif i == 0:
                    tail_cp[gn - NPOS].start(priority=_BG)
                fg[g][i](m, sem.at[gn % _NS]).start(priority=_FG)

            hh, j = g // 8, g % _NG
            if (g % 8) < _NG:
                s = _dot(q_scr[hh].astype(BF16), kbuf[j])
                s_parts.append(_rbf(_rbf(s) * scale))
                if j == _NG - 1:
                    s = jnp.concatenate(s_parts, axis=1)
                    s_parts = []
                    e = jnp.exp(s - jnp.max(s, axis=-1, keepdims=True))
                    l = jnp.sum(e, axis=-1, keepdims=True)
                    p_scr[...] = _rbf(e * (1.0 / l))
                    acc = jnp.zeros((DH // 8, 8, 128), F32)
                    if hh == 1 and not last:
                        project_q()
            else:
                for t in range(GW // 256):
                    vt = vbuf[j, :, t * 256:(t + 1) * 256].astype(F32)
                    pj = p_scr[:, j * GW + t * 256:j * GW + (t + 1) * 256]
                    prod = vt.reshape(DH // 8, 8, 256) * pj[None]
                    acc = acc + prod[:, :, 0:128] + prod[:, :, 128:256]
                if j == _NG - 1:
                    o = _rbf(jnp.sum(acc, axis=-1, keepdims=True))
                    woh = wo[hh].astype(F32).reshape(DH // 8, 8, D)
                    attn8 = attn8 + jnp.sum(woh * o, axis=0)
            if last and g in (4, 5, 6, 8):
                k = 2 + len(mods)
                mods.append(_rbf(_dot(sc8, wm[:, k * D:(k + 1) * D])))
        return (attn8, mods) if last else attn8

    attn8 = lax.fori_loop(0, NP - 1, lambda m, a: pair_body(m, a, False),
                          jnp.zeros((8, D), F32))
    attn8, (ga, sb, cb, gb) = pair_body(NP - 1, attn8, True)
    attn = _rbf(jnp.sum(attn8, axis=0, keepdims=True))

    x1 = _rbf(x + _rbf(ga * attn))
    h2 = (_rbf(_rbf(_layernorm_rows(x1)) * _rbf(1.0 + cb)) + sb).astype(BF16)
    g_ = _rbf(_dot(h2, wg[...]))
    u_ = _rbf(_dot(h2, wu[...]))
    hh_ = (g_ * u_).astype(BF16)
    y = None
    spans = [(0, 320 + 64, wd_tail[0]), (384, 64, wd_tail[1]), (448, 64, wd_tail[2])]
    for t in range(LA):
        for i in range(_TPG):
            fg_last[NPOS - LA + t][i](NP - 1, sem.at[(NPOS + t) % _NS]).wait()
        tail_cp[t].wait()
        for r0, n in (spans[t][:2], spans[t][2]):
            part = _dot(hh_[:, r0:r0 + n], wd[r0:r0 + n, :])
            y = part if y is None else y + part
    x2 = x1 + _rbf(gb * _rbf(y))
    out_ref[...] = x2[0:1, :].astype(out_ref.dtype)


@jax.jit
def pallas_adaLN_cond__sliding_block_cached__glu_gated_bilinear__decode_kernel(
    A_x: jax.Array,
    A_k_cache: jax.Array,
    A_v_cache: jax.Array,
    A_wq: jax.Array,
    A_wo: jax.Array,
    B_x: jax.Array,
    B_w_gate: jax.Array,
    B_w_up: jax.Array,
    B_w_down: jax.Array,
    c: jax.Array,
    w_mod: jax.Array,
):
    B, SQ, D = A_x.shape
    _, HKV, SK, DH = A_k_cache.shape
    W = min(4096, max(256, SK // 4))
    FF = B_w_gate.shape[1]
    assert B == 1 and SQ == 1 and HKV == _HQ and DH == _DH
    assert (D, FF, W) == (640, 1536, _NG * _TPG * _CW)

    kt = jnp.swapaxes(A_k_cache, 2, 3).reshape(HKV * DH, SK)
    vt = jnp.swapaxes(A_v_cache, 2, 3).reshape(HKV * DH, SK)
    x2d = A_x.reshape(1, D)

    any_spec = pl.BlockSpec(memory_space=pl.ANY)
    out = pl.pallas_call(
        functools.partial(_kernel, D=D, FF=FF, SK=SK, W=W),
        out_shape=jax.ShapeDtypeStruct((1, D), A_x.dtype),
        in_specs=[any_spec] * 10,
        out_specs=pl.BlockSpec(memory_space=pltpu.VMEM),
        scratch_shapes=[
            pltpu.VMEM((1, D), BF16),
            pltpu.VMEM((1, D), BF16),
            pltpu.VMEM((_NG, DH, _TPG * _CW), BF16),
            pltpu.VMEM((_NG, DH, _TPG * _CW), BF16),
            pltpu.VMEM((D, 2 * DH), BF16),
            pltpu.VMEM((2, DH, D), BF16),
            pltpu.VMEM(B_w_gate.shape, BF16),
            pltpu.VMEM(B_w_up.shape, BF16),
            pltpu.VMEM(B_w_down.shape, BF16),
            pltpu.VMEM(w_mod.shape, BF16),
            pltpu.VMEM((2, 8, DH), F32),
            pltpu.VMEM((8, D), F32),
            pltpu.VMEM((8, W), F32),
            pltpu.SemaphoreType.DMA((_NS,)),
            pltpu.SemaphoreType.DMA((1,)),
        ],
        compiler_params=pltpu.CompilerParams(
            vmem_limit_bytes=64 * 1024 * 1024, disable_bounds_checks=True),
    )(x2d, c, kt, vt, A_wq, A_wo, B_w_gate, B_w_up, B_w_down, w_mod)
    return out.reshape(B, SQ, D)
```

```python
import functools

import jax
import jax.numpy as jnp
import numpy as np
from jax import lax
import jax.experimental.pallas as pl
import jax.experimental.pallas.tpu as pltpu

F32 = jnp.float32
BF16 = jnp.bfloat16

_HQ = 32
_DH = 192
_EPS = 1e-5

_CW = 128
_TPG = 8
_NG = 4
_NS = 4
_BG, _FG = 1, 0
_WM_S, _WM_C = 8, 384
_WQ_S, _WQ_C = 10, 256


def _rbf(v):
    return v.astype(BF16).astype(F32)


def _layernorm_rows(v):
    m = jnp.mean(v, axis=-1, keepdims=True)
    d = v - m
    var = jnp.mean(d * d, axis=-1, keepdims=True)
    return d * lax.rsqrt(var + _EPS)


def _dot(a, b):
    return jnp.dot(a, b, preferred_element_type=F32)


def _split(items, n):
    k = len(items)
    return [items[(i * k) // n:((i + 1) * k) // n] for i in range(n)]


def _kernel(x_hbm, c_hbm, kt_hbm, vt_hbm, wq_hbm, wo_hbm, wg_hbm, wu_hbm, wd_hbm, wm_hbm,
            out_ref,
            xbuf, cbuf, kbuf, vbuf, wq, wo, wg, wu, wd, wm, q_scr, h_scr, mod_scr, p_scr,
            sem,
            *, D, FF, SK, W):
    H, DH = _HQ, _DH
    GW = _CW * _TPG
    NP = H // 2
    NPOS = 4 * _NG
    LA = _NS - 1
    RB = D // NP
    c0 = SK - W
    scale = float(np.asarray(DH ** -0.5, dtype=BF16))
    cp = pltpu.make_async_copy

    def mul(v, k, a=8):
        return v * k if isinstance(v, int) else pl.multiple_of(v * k, a)

    def same(src, dst, idx):
        return lambda s: cp(src.at[idx], dst.at[idx], s)

    def run_group(bg, fg, s, nbg, nfg, ns):
        for f in fg:
            f(s).wait()
        for b, nb, nf in zip(bg, _split(nbg, len(bg)), _split(nfg, len(bg))):
            b(s).wait()
            for f in nb:
                f(ns).start(priority=_BG)
            for f in nf:
                f(ns).start(priority=_FG)

    def kv_group(m, g):
        src, dst = (kt_hbm, kbuf) if (g % 8) < _NG else (vt_hbm, vbuf)
        j = g % _NG

        def piece(i):
            return lambda s: cp(
                src.at[pl.ds(mul(m, 2 * DH) + (g // 8) * DH, DH), pl.ds(c0 + j * GW + i * _CW, _CW)],
                dst.at[j, :, pl.ds(i * _CW, _CW)], s)
        return [piece(i) for i in range(_TPG)]

    def wo_pieces(m, hh):
        def piece(r, col, n):
            return lambda s: cp(
                wo_hbm.at[pl.ds(mul(m, 2 * DH) + hh * DH + 8 * r, 8), pl.ds(col, n)],
                wo.at[hh, pl.ds(8 * r, 8), pl.ds(col, n)], s)
        return [piece(r, col, n) for r in range(DH // 8) for col, n in ((0, 384), (384, D - 384))]

    def ffn_pieces(m):
        out = []
        for src, dst in ((wg_hbm, wg), (wu_hbm, wu)):
            for r in range(RB // 8):
                for col in range(0, FF, 512):
                    out.append(lambda s, src=src, dst=dst, r=r, col=col: same(
                        src, dst, (pl.ds(mul(m, RB) + 8 * r, 8), pl.ds(col, 512)))(s))
        for r in range(2):
            out.append(lambda s, r=r: same(wd_hbm, wd, (pl.ds(mul(m, 16) + 8 * r, 8), slice(None)))(s))
        return out

    def wd_rows(r0, n):
        return same(wd_hbm, wd, (pl.ds(r0, n), slice(None)))

    def pair_fg(m):
        flat = wo_pieces(m, 0) + wo_pieces(m, 1) + ffn_pieces(m)
        assert len(flat) == NPOS * _TPG
        return _split(flat, NPOS)

    tail_k = [16 * NP, 896, 1408, FF]
    tail_fg = [[wd_rows(tail_k[t] + 8 * i, 8) for i in range(_TPG)] for t in range(LA)]
    tail_bg = [[wd_rows(tail_k[t] + 8 * _TPG, tail_k[t + 1] - tail_k[t] - 8 * _TPG)] for t in range(LA)]

    mr, qr = wm.shape[1] // 8, wq.shape[1] // 8
    s_bg = [[same(wm_hbm, wm, (slice(None), pl.ds(8 * r, 8), pl.ds(col, _WM_C)))
             for col in range(0, 6 * D, _WM_C)] for r in range(mr - 1)]
    n_wm = len(s_bg)
    for r in range(qr - 1):
        s_bg += _split([same(wq_hbm, wq, (slice(None), pl.ds(8 * r, 8), pl.ds(col, _WQ_C)))
                        for col in range(0, H * DH, _WQ_C)], 3)
    n_s = len(s_bg)
    wm_fg = [same(wm_hbm, wm, (st, pl.ds(8 * (mr - 1), 8), pl.ds(col, 384)))
             for st in range(_WM_S) for col in range(0, 6 * D, 384)]
    wq_fg = [same(wq_hbm, wq, (st, pl.ds(8 * (qr - 1), 8), pl.ds(col, 384)))
             for st in range(_WQ_S) for col in range(0, H * DH, 384)]
    rest = wm_fg + wq_fg
    n_slots = sum(len(s_bg[g]) for g in range(n_s - LA))
    extra = len(rest) - n_slots
    s_fg = [[lambda s: cp(c_hbm, cbuf, s), lambda s: cp(x_hbm, xbuf, s)] + rest[:extra], [], []]
    pos = extra
    wm_done = None
    for g in range(LA, n_s):
        s_fg.append(rest[pos:pos + len(s_bg[g - LA])])
        pos += len(s_bg[g - LA])
        if wm_done is None and pos >= len(wm_fg):
            wm_done = max(g, n_wm - 1)
    off = (-n_s) % _NS
    ssem = lambda g: sem.at[(g + off) % _NS]

    for g in range(LA):
        for f in s_fg[g]:
            f(ssem(g)).start(priority=_FG)
        for f in s_bg[g]:
            f(ssem(g)).start(priority=_BG)

    def project_q(m):
        w2 = wq[:, :, pl.ds(mul(m, 2 * DH, 128), 2 * DH)].reshape(D, 2 * DH)
        q2 = _dot(h_scr[...].astype(BF16), w2)
        q_scr[0] = q2[:, 0:DH]
        q_scr[1] = q2[:, DH:2 * DH]

    def load_x():
        return jnp.broadcast_to(xbuf[...].astype(F32), (8, D))

    fg0 = pair_fg(0)
    for g in range(n_s):
        gn = g + LA
        nbg, nfg = (s_bg[gn], s_fg[gn]) if gn < n_s else (kv_group(0, gn - n_s), fg0[gn - n_s])
        run_group(s_bg[g], s_fg[g], ssem(g), nbg, nfg, ssem(gn))
        k = g - wm_done
        if 0 <= k < 6:
            c = cbuf[...].astype(F32)
            sc = c * (1.0 / (1.0 + jnp.exp(-c)))
            sc8 = jnp.broadcast_to(sc, (8, D)).astype(BF16)
            wk = wm[:, :, k * D:(k + 1) * D].reshape(D, D)
            mod_scr[:, k * D:(k + 1) * D] = _rbf(_dot(sc8, wk))
        elif k == 6:
            sa, ca = mod_scr[:, 0:D], mod_scr[:, D:2 * D]
            h_scr[...] = _rbf(_rbf(_layernorm_rows(load_x())) * _rbf(1.0 + ca)) + sa
    project_q(0)

    def pair_body(m, attn8, last):
        fg = pair_fg(m)
        fg_next = None if last else pair_fg(m + 1)
        s_parts, acc = [], None
        for g in range(NPOS):
            gn = g + LA
            if gn < NPOS:
                nbg, nfg = kv_group(m, gn), fg[gn]
            elif not last:
                nbg, nfg = kv_group(m + 1, gn - NPOS), fg_next[gn - NPOS]
            else:
                nbg, nfg = tail_bg[gn - NPOS], tail_fg[gn - NPOS]
                nbg = nbg + [None] * 0
            if last and gn >= NPOS:
                for f in fg[g]:
                    f(sem.at[g % _NS]).wait()
                for i, b in enumerate(kv_group(m, g)):
                    b(sem.at[g % _NS]).wait()
                    if i == 0:
                        nbg[0](sem.at[gn % _NS]).start(priority=_BG)
                    nfg[i](sem.at[gn % _NS]).start(priority=_FG)
            else:
                run_group(kv_group(m, g), fg[g], sem.at[g % _NS], nbg, nfg, sem.at[gn % _NS])

            hh, j = g // 8, g % _NG
            if (g % 8) < _NG:
                s = _dot(q_scr[hh].astype(BF16), kbuf[j])
                s_parts.append(_rbf(_rbf(s) * scale))
                if j == _NG - 1:
                    s = jnp.concatenate(s_parts, axis=1)
                    s_parts = []
                    e = jnp.exp(s - jnp.max(s, axis=-1, keepdims=True))
                    l = jnp.sum(e, axis=-1, keepdims=True)
                    p_scr[...] = _rbf(e * (1.0 / l))
                    acc = jnp.zeros((DH // 8, 8, 128), F32)
                    if hh == 1 and not last:
                        project_q(m + 1)
            else:
                for t in range(GW // 256):
                    vt = vbuf[j, :, t * 256:(t + 1) * 256].astype(F32)
                    pj = p_scr[:, j * GW + t * 256:j * GW + (t + 1) * 256]
                    prod = vt.reshape(DH // 8, 8, 256) * pj[None]
                    acc = acc + prod[:, :, 0:128] + prod[:, :, 128:256]
                if j == _NG - 1:
                    o = _rbf(jnp.sum(acc, axis=-1, keepdims=True))
                    woh = wo[hh].astype(F32).reshape(DH // 8, 8, D)
                    attn8 = attn8 + jnp.sum(woh * o, axis=0)
        return attn8

    attn8 = lax.fori_loop(0, NP - 1, lambda m, a: pair_body(m, a, False),
                          jnp.zeros((8, D), F32))
    attn8 = pair_body(NP - 1, attn8, True)
    attn = _rbf(jnp.sum(attn8, axis=0, keepdims=True))

    ga, sb, cb, gb = [mod_scr[:, k * D:(k + 1) * D] for k in range(2, 6)]
    x1 = _rbf(load_x() + _rbf(ga * attn))
    h2 = (_rbf(_rbf(_layernorm_rows(x1)) * _rbf(1.0 + cb)) + sb).astype(BF16)
    g_ = _rbf(_dot(h2, wg[...]))
    u_ = _rbf(_dot(h2, wu[...]))
    hh_ = (g_ * u_).astype(BF16)
    y = None
    for t in range(LA):
        for f in tail_fg[t] + tail_bg[t]:
            f(sem.at[(NPOS + t) % _NS]).wait()
        r0, r1 = (0 if t == 0 else tail_k[t]), tail_k[t + 1]
        part = _dot(hh_[:, r0:r1], wd[r0:r1, :])
        y = part if y is None else y + part
    x2 = x1 + _rbf(gb * _rbf(y))
    out_ref[...] = x2[0:1, :].astype(out_ref.dtype)


@jax.jit
def pallas_adaLN_cond__sliding_block_cached__glu_gated_bilinear__decode_kernel(
    A_x: jax.Array,
    A_k_cache: jax.Array,
    A_v_cache: jax.Array,
    A_wq: jax.Array,
    A_wo: jax.Array,
    B_x: jax.Array,
    B_w_gate: jax.Array,
    B_w_up: jax.Array,
    B_w_down: jax.Array,
    c: jax.Array,
    w_mod: jax.Array,
):
    B, SQ, D = A_x.shape
    _, HKV, SK, DH = A_k_cache.shape
    W = min(4096, max(256, SK // 4))
    FF = B_w_gate.shape[1]
    assert B == 1 and SQ == 1 and HKV == _HQ and DH == _DH
    assert (D, FF, W) == (640, 1536, _NG * _TPG * _CW)

    kt = jnp.swapaxes(A_k_cache, 2, 3).reshape(HKV * DH, SK)
    vt = jnp.swapaxes(A_v_cache, 2, 3).reshape(HKV * DH, SK)
    x2d = A_x.reshape(1, D)
    wq3 = A_wq.reshape(_WQ_S, D // _WQ_S, HKV * DH)
    wm3 = w_mod.reshape(_WM_S, D // _WM_S, 6 * D)

    any_spec = pl.BlockSpec(memory_space=pl.ANY)
    out = pl.pallas_call(
        functools.partial(_kernel, D=D, FF=FF, SK=SK, W=W),
        out_shape=jax.ShapeDtypeStruct((1, D), A_x.dtype),
        in_specs=[any_spec] * 10,
        out_specs=pl.BlockSpec(memory_space=pltpu.VMEM),
        scratch_shapes=[
            pltpu.VMEM((1, D), BF16),
            pltpu.VMEM((1, D), BF16),
            pltpu.VMEM((_NG, DH, _TPG * _CW), BF16),
            pltpu.VMEM((_NG, DH, _TPG * _CW), BF16),
            pltpu.VMEM(wq3.shape, BF16),
            pltpu.VMEM((2, DH, D), BF16),
            pltpu.VMEM(B_w_gate.shape, BF16),
            pltpu.VMEM(B_w_up.shape, BF16),
            pltpu.VMEM(B_w_down.shape, BF16),
            pltpu.VMEM(wm3.shape, BF16),
            pltpu.VMEM((2, 8, DH), F32),
            pltpu.VMEM((8, D), F32),
            pltpu.VMEM((8, 6 * D), F32),
            pltpu.VMEM((8, W), F32),
            pltpu.SemaphoreType.DMA((_NS,)),
        ],
        compiler_params=pltpu.CompilerParams(
            vmem_limit_bytes=64 * 1024 * 1024, disable_bounds_checks=True),
    )(x2d, c, kt, vt, wq3, A_wo, B_w_gate, B_w_up, B_w_down, wm3)
    return out.reshape(B, SQ, D)
```

```python
import functools

import jax
import jax.numpy as jnp
import numpy as np
from jax import lax
import jax.experimental.pallas as pl
import jax.experimental.pallas.tpu as pltpu

F32 = jnp.float32
BF16 = jnp.bfloat16

_HQ = 32
_DH = 192
_EPS = 1e-5

_CW = 128
_TPG = 8
_NG = 4
_NS = 4
_BG, _FG = 1, 0
_TAIL_K = (896, 1344, 1488)
_N_VPU = 2
_HC = 256
_WM_S, _WM_C = 8, 384
_WQ_S, _WQ_C = 10, 256


def _rbf(v):
    return v.astype(BF16).astype(F32)


def _layernorm_rows(v):
    m = jnp.mean(v, axis=-1, keepdims=True)
    d = v - m
    var = jnp.mean(d * d, axis=-1, keepdims=True)
    return d * lax.rsqrt(var + _EPS)


def _dot(a, b):
    return jnp.dot(a, b, preferred_element_type=F32)


def _split(items, n):
    k = len(items)
    return [items[(i * k) // n:((i + 1) * k) // n] for i in range(n)]


def _kernel(x_hbm, c_hbm, kt_hbm, vt_hbm, wq_hbm, wo_hbm, wg_hbm, wu_hbm, wd_hbm, wm_hbm,
            out_ref,
            xbuf, cbuf, kbuf, vbuf, wq, wo, wg, wu, wd, wm, q_scr, h_scr, mod_scr, p_scr, hc_scr, z_scr,
            sem,
            *, D, FF, SK, W):
    H, DH = _HQ, _DH
    GW = _CW * _TPG
    NP = H // 2
    NPOS = 4 * _NG
    LA = _NS - 1
    RB = D // NP
    c0 = SK - W
    scale = float(np.asarray(DH ** -0.5, dtype=BF16))
    cp = pltpu.make_async_copy

    def mul(v, k, a=8):
        return v * k if isinstance(v, int) else pl.multiple_of(v * k, a)

    def same(src, dst, idx):
        return lambda s: cp(src.at[idx], dst.at[idx], s)

    def run_group(bg, fg, s, nbg, nfg, ns):
        for f in fg:
            f(s).wait()
        for b, nb, nf in zip(bg, _split(nbg, len(bg)), _split(nfg, len(bg))):
            b(s).wait()
            for f in nb:
                f(ns).start(priority=_BG)
            for f in nf:
                f(ns).start(priority=_FG)

    def kv_group(m, g):
        src, dst = (kt_hbm, kbuf) if (g % 8) < _NG else (vt_hbm, vbuf)
        j = g % _NG

        def piece(i):
            return lambda s: cp(
                src.at[pl.ds(mul(m, 2 * DH) + (g // 8) * DH, DH), pl.ds(c0 + j * GW + i * _CW, _CW)],
                dst.at[j, :, pl.ds(i * _CW, _CW)], s)
        return [piece(i) for i in range(_TPG)]

    def wo_pieces(m, hh):
        def piece(r, col, n):
            return lambda s: cp(
                wo_hbm.at[pl.ds(mul(m, 2 * DH) + hh * DH + 8 * r, 8), pl.ds(col, n)],
                wo.at[hh, pl.ds(8 * r, 8), pl.ds(col, n)], s)
        return [piece(r, col, n) for r in range(DH // 8) for col, n in ((0, 384), (384, D - 384))]

    def ffn_pieces(m):
        out = []
        for src, dst in ((wg_hbm, wg), (wu_hbm, wu)):
            for r in range(RB // 8):
                for col in range(0, FF, 512):
                    out.append(lambda s, src=src, dst=dst, r=r, col=col: same(
                        src, dst, (pl.ds(mul(m, RB) + 8 * r, 8), pl.ds(col, 512)))(s))
        return out

    def wd_rows(r0, n):
        return same(wd_hbm, wd, (pl.ds(r0, n), slice(None)))

    def pair_fg(m):
        flat = wo_pieces(m, 0) + wo_pieces(m, 1) + ffn_pieces(m)
        return _split(flat[:96], 12) + _split(flat[96:], 4)

    tail_k = _TAIL_K + (FF,)
    n_tf = LA * _TPG
    tail_fg = [wd_rows(8 * i, 8) for i in range(n_tf)]
    tail_sem = [sem.at[NPOS % _NS]] + [sem.at[_NS + t] for t in range(len(_TAIL_K))]
    tail_bg = [wd_rows(a, b - a) for a, b in zip((8 * n_tf,) + tail_k[:-1], tail_k)]

    mr, qr = wm.shape[1] // 8, wq.shape[1] // 8
    s_bg = [[same(wm_hbm, wm, (slice(None), pl.ds(8 * r, 8), pl.ds(col, _WM_C)))
             for col in range(0, 6 * D, _WM_C)] for r in range(mr - 1)]
    n_wm = len(s_bg)
    for r in range(qr - 1):
        s_bg += _split([same(wq_hbm, wq, (slice(None), pl.ds(8 * r, 8), pl.ds(col, _WQ_C)))
                        for col in range(0, H * DH, _WQ_C)], 3)
    n_s = len(s_bg)
    wm_fg = [same(wm_hbm, wm, (st, pl.ds(8 * (mr - 1), 8), pl.ds(col, 384)))
             for st in range(_WM_S) for col in range(0, 6 * D, 384)]
    wq_fg = [same(wq_hbm, wq, (st, pl.ds(8 * (qr - 1), 8), pl.ds(col, 384)))
             for st in range(_WQ_S) for col in range(0, H * DH, 384)]
    rest = wm_fg + wq_fg
    n_slots = sum(len(s_bg[g]) for g in range(n_s - LA))
    extra = len(rest) - n_slots
    s_fg = [[lambda s: cp(c_hbm, cbuf, s), lambda s: cp(x_hbm, xbuf, s)] + rest[:extra], [], []]
    pos = extra
    wm_done = None
    for g in range(LA, n_s):
        s_fg.append(rest[pos:pos + len(s_bg[g - LA])])
        pos += len(s_bg[g - LA])
        if wm_done is None and pos >= len(wm_fg):
            wm_done = max(g, n_wm - 1)
    off = (-n_s) % _NS
    ssem = lambda g: sem.at[(g + off) % _NS]

    for g in range(LA):
        for f, ff in zip(s_bg[g], _split(s_fg[g], len(s_bg[g]))):
            f(ssem(g)).start(priority=_BG)
            for f2 in ff:
                f2(ssem(g)).start(priority=_FG)

    def project_q(m):
        w2 = wq[:, :, pl.ds(mul(m, 2 * DH, 128), 2 * DH)].reshape(D, 2 * DH)
        q2 = _dot(h_scr[...].astype(BF16), w2)
        q_scr[0] = q2[:, 0:DH]
        q_scr[1] = q2[:, DH:2 * DH]

    def load_x():
        return jnp.broadcast_to(xbuf[...].astype(F32), (8, D))

    fg0 = pair_fg(0)
    for g in range(n_s):
        gn = g + LA
        nbg, nfg = (s_bg[gn], s_fg[gn]) if gn < n_s else (kv_group(0, gn - n_s), fg0[gn - n_s])
        run_group(s_bg[g], s_fg[g], ssem(g), nbg, nfg, ssem(gn))
        k = g - wm_done
        if 0 <= k < 6:
            c = cbuf[...].astype(F32)
            sc = c * (1.0 / (1.0 + jnp.exp(-c)))
            sc8 = jnp.broadcast_to(sc, (8, D)).astype(BF16)
            wk = wm[:, :, k * D:(k + 1) * D].reshape(D, D)
            mod_scr[:, k * D:(k + 1) * D] = _rbf(_dot(sc8, wk))
        elif k == 6:
            sa, ca = mod_scr[:, 0:D], mod_scr[:, D:2 * D]
            h_scr[...] = _rbf(_rbf(_layernorm_rows(load_x())) * _rbf(1.0 + ca)) + sa
    project_q(0)

    def pair_body(m, attn8, last):
        fg = pair_fg(m)
        fg_next = None if last else pair_fg(m + 1)
        s_parts, acc = [], None
        for g in range(NPOS):
            gn = g + LA
            if gn < NPOS:
                nbg, nfg = kv_group(m, gn), fg[gn]
            elif not last:
                nbg, nfg = kv_group(m + 1, gn - NPOS), fg_next[gn - NPOS]
            if last and gn >= NPOS:
                for f in fg[g]:
                    f(sem.at[g % _NS]).wait()
                for i, b in enumerate(kv_group(m, g)):
                    b(sem.at[g % _NS]).wait()
                    k = (gn - NPOS) * _TPG + i
                    if k < len(tail_bg):
                        tail_bg[k](tail_sem[k]).start(priority=_BG)
                    tail_fg[k](tail_sem[0]).start(priority=_FG)
            else:
                run_group(kv_group(m, g), fg[g], sem.at[g % _NS], nbg, nfg, sem.at[gn % _NS])

            hh, j = g // 8, g % _NG
            if (g % 8) < _NG:
                s = _dot(q_scr[hh].astype(BF16), kbuf[j])
                s_parts.append(_rbf(_rbf(s) * scale))
                if j == _NG - 1:
                    s = jnp.concatenate(s_parts, axis=1)
                    s_parts = []
                    e = jnp.exp(s - jnp.max(s, axis=-1, keepdims=True))
                    l = jnp.sum(e, axis=-1, keepdims=True)
                    p_scr[...] = _rbf(e * (1.0 / l))
                    acc = jnp.zeros((DH // 8, 8, 128), F32)
                    if hh == 1 and not last:
                        project_q(m + 1)
            else:
                for t in range(GW // 256):
                    vt = vbuf[j, :, t * 256:(t + 1) * 256].astype(F32)
                    pj = p_scr[:, j * GW + t * 256:j * GW + (t + 1) * 256]
                    prod = vt.reshape(DH // 8, 8, 256) * pj[None]
                    acc = acc + prod[:, :, 0:128] + prod[:, :, 128:256]
                if j == _NG - 1:
                    o = _rbf(jnp.sum(acc, axis=-1, keepdims=True))
                    woh = wo[hh].astype(F32).reshape(DH // 8, 8, D)
                    attn8 = attn8 + jnp.sum(woh * o, axis=0)
        return attn8

    attn8 = lax.fori_loop(0, NP - 1, lambda m, a: pair_body(m, a, False),
                          jnp.zeros((8, D), F32))
    attn8 = pair_body(NP - 1, attn8, True)
    attn = _rbf(jnp.sum(attn8, axis=0, keepdims=True))

    ga, sb, cb, gb = [mod_scr[:, k * D:(k + 1) * D] for k in range(2, 6)]
    x1 = _rbf(load_x() + _rbf(ga * attn))
    h2 = (_rbf(_rbf(_layernorm_rows(x1)) * _rbf(1.0 + cb)) + sb).astype(BF16)
    g_ = _rbf(_dot(h2, wg[...]))
    u_ = _rbf(_dot(h2, wu[...]))
    hh_ = (g_ * u_).astype(BF16)
    if _N_VPU:
        hc0 = FF - _HC
        hc_scr[...] = jnp.broadcast_to(hh_[0:1, hc0:FF].astype(F32), (128, _HC)).T
    for f in tail_fg:
        f(tail_sem[0]).wait()
    n_t = len(tail_bg)
    for t in range(n_t):
        tail_bg[t](tail_sem[t]).wait()
        r0, r1 = (0 if t == 0 else tail_k[t - 1]), tail_k[t]
        if t < n_t - _N_VPU:
            y = _dot(hh_[:, r0:r1], wd[r0:r1, :])
            if t > 0:
                y = y + h_scr[...]
            if t < n_t - 1:
                h_scr[...] = y
        else:
            n = (r1 - r0) // 8
            hc = hc_scr[r0 - hc0:r1 - hc0, :].reshape(n, 8, 128)
            hc = jnp.concatenate([hc] * (D // 128), axis=-1)
            z = jnp.sum(wd[r0:r1, :].astype(F32).reshape(n, 8, D) * hc, axis=0)
            if t > n_t - _N_VPU:
                z = z + z_scr[...]
            if t < n_t - 1:
                z_scr[...] = z
            else:
                y = h_scr[...] + jnp.sum(z, axis=0, keepdims=True)
    x2 = x1 + _rbf(gb * _rbf(y))
    out_ref[...] = x2[0:1, :].astype(out_ref.dtype)


@jax.jit
def pallas_adaLN_cond__sliding_block_cached__glu_gated_bilinear__decode_kernel(
    A_x: jax.Array,
    A_k_cache: jax.Array,
    A_v_cache: jax.Array,
    A_wq: jax.Array,
    A_wo: jax.Array,
    B_x: jax.Array,
    B_w_gate: jax.Array,
    B_w_up: jax.Array,
    B_w_down: jax.Array,
    c: jax.Array,
    w_mod: jax.Array,
):
    B, SQ, D = A_x.shape
    _, HKV, SK, DH = A_k_cache.shape
    W = min(4096, max(256, SK // 4))
    FF = B_w_gate.shape[1]
    assert B == 1 and SQ == 1 and HKV == _HQ and DH == _DH
    assert (D, FF, W) == (640, 1536, _NG * _TPG * _CW)

    kt = jnp.swapaxes(A_k_cache, 2, 3).reshape(HKV * DH, SK)
    vt = jnp.swapaxes(A_v_cache, 2, 3).reshape(HKV * DH, SK)
    x2d = A_x.reshape(1, D)
    wq3 = A_wq.reshape(_WQ_S, D // _WQ_S, HKV * DH)
    wm3 = w_mod.reshape(_WM_S, D // _WM_S, 6 * D)

    any_spec = pl.BlockSpec(memory_space=pl.ANY)
    out = pl.pallas_call(
        functools.partial(_kernel, D=D, FF=FF, SK=SK, W=W),
        out_shape=jax.ShapeDtypeStruct((1, D), A_x.dtype),
        in_specs=[any_spec] * 10,
        out_specs=pl.BlockSpec(memory_space=pltpu.VMEM),
        scratch_shapes=[
            pltpu.VMEM((1, D), BF16),
            pltpu.VMEM((1, D), BF16),
            pltpu.VMEM((_NG, DH, _TPG * _CW), BF16),
            pltpu.VMEM((_NG, DH, _TPG * _CW), BF16),
            pltpu.VMEM(wq3.shape, BF16),
            pltpu.VMEM((2, DH, D), BF16),
            pltpu.VMEM(B_w_gate.shape, BF16),
            pltpu.VMEM(B_w_up.shape, BF16),
            pltpu.VMEM(B_w_down.shape, BF16),
            pltpu.VMEM(wm3.shape, BF16),
            pltpu.VMEM((2, 8, DH), F32),
            pltpu.VMEM((8, D), F32),
            pltpu.VMEM((8, 6 * D), F32),
            pltpu.VMEM((8, W), F32),
            pltpu.VMEM((_HC, 128), F32),
            pltpu.VMEM((8, D), F32),
            pltpu.SemaphoreType.DMA((_NS + len(_TAIL_K),)),
        ],
        compiler_params=pltpu.CompilerParams(
            vmem_limit_bytes=64 * 1024 * 1024, disable_bounds_checks=True,
            disable_semaphore_checks=True),
    )(x2d, c, kt, vt, wq3, A_wo, B_w_gate, B_w_up, B_w_down, wm3)
    return out.reshape(B, SQ, D)
```

```python
import dataclasses
import functools

import jax
import jax.numpy as jnp
import numpy as np
from jax import lax
import jax.experimental.pallas as pl
import jax.experimental.pallas.tpu as pltpu

F32 = jnp.float32
BF16 = jnp.bfloat16

_HQ = 32
_DH = 192
_EPS = 1e-5

_CW = 128
_TPG = 8
_NG = 4
_NS = 4
_LA = 3
_MID = 3
_BG, _FG = 1, 0
_WM_S, _WM_C = 8, 384
_WQ_S, _WQ_C = 10, 256
_WQ_F = 256
_WD_E = 2
_TAIL_K = (1024, 1344, 1488)
_N_VPU = 2
_HC = 256


def _rbf(v):
    return v.astype(BF16).astype(F32)


def _layernorm_rows(v):
    m = jnp.mean(v, axis=-1, keepdims=True)
    d = v - m
    var = jnp.mean(d * d, axis=-1, keepdims=True)
    return d * lax.rsqrt(var + _EPS)


def _dot(a, b):
    return jnp.dot(a, b, preferred_element_type=F32)


def _split(items, n):
    k = len(items)
    return [items[(i * k) // n:((i + 1) * k) // n] for i in range(n)]


def _kernel(x_hbm, c_hbm, kt_hbm, vt_hbm, wq_hbm, wo_hbm, wg_hbm, wu_hbm, wd_hbm, wm_hbm,
            out_ref,
            xbuf, cbuf, kbuf, vbuf, wq, wo, wg, wu, wd, wm,
            q_scr, h_scr, mod_scr, p_scr, hc_scr, z_scr, sem,
            *, D, FF, SK, W):
    H, DH, LA = _HQ, _DH, _LA
    GW = _CW * _TPG
    NP = H // 2
    NPOS = 4 * _NG
    RB = D // NP
    c0 = SK - W
    scale = float(np.asarray(DH ** -0.5, dtype=BF16))
    cp = pltpu.make_async_copy

    def mul(v, k, a=8):
        return v * k if isinstance(v, int) else pl.multiple_of(v * k, a)

    def same(src, dst, idx):
        return lambda s: cp(src.at[idx], dst.at[idx], s)

    def run_group(bg, fg, s, issue, mid=None):
        for f in fg:
            f(s).wait()
        for i, b in enumerate(bg):
            b(s).wait()
            for f, ns, prio in issue[i]:
                f(ns).start(priority=prio)
            if mid is not None and i == _MID:
                mid()

    def plan(n, nbg, nfg, ns):
        return [[(f, ns, _BG) for f in b] + [(f, ns, _FG) for f in g]
                for b, g in zip(_split(nbg, n), _split(nfg, n))]

    def kv_group(m, g):
        src, dst = (kt_hbm, kbuf) if (g % 8) < _NG else (vt_hbm, vbuf)
        j = g % _NG

        def piece(i):
            return lambda s: cp(
                src.at[pl.ds(mul(m, 2 * DH) + (g // 8) * DH, DH), pl.ds(c0 + j * GW + i * _CW, _CW)],
                dst.at[j, :, pl.ds(i * _CW, _CW)], s)
        return [piece(i) for i in range(_TPG)]

    def wo_pieces(m, hh):
        def piece(r, col, n):
            return lambda s: cp(
                wo_hbm.at[pl.ds(mul(m, 2 * DH) + hh * DH + 8 * r, 8), pl.ds(col, n)],
                wo.at[hh, pl.ds(8 * r, 8), pl.ds(col, n)], s)
        return [piece(r, col, n) for r in range(DH // 8) for col, n in ((0, 384), (384, D - 384))]

    def ffn_pieces(m):
        def piece(src, dst, k, r, cols):
            return lambda s: same(src, dst, (pl.ds(mul(m, k) + 8 * r, 8), cols))(s)
        out = [piece(src, dst, RB, r, pl.ds(col, 512))
               for src, dst in ((wg_hbm, wg), (wu_hbm, wu))
               for r in range(RB // 8) for col in range(0, FF, 512)]
        return out + [piece(wd_hbm, wd, 8 * _WD_E, r, slice(None)) for r in range(_WD_E)]

    def pair_fg(m):
        wos = _split(wo_pieces(m, 0), 8) + _split(wo_pieces(m, 1), 8)
        ffs = _split(ffn_pieces(m), NPOS)
        return [w[:3] + f[:1] + w[3:] + f[1:] for w, f in zip(wos, ffs)]

    def wd_rows(r0, n):
        return same(wd_hbm, wd, (pl.ds(r0, n), slice(None)))

    tail_k = _TAIL_K + (FF,)
    e0, n_tf = 8 * _WD_E * NP, LA * _TPG
    tail_fg = [wd_rows(e0 + 8 * i, 8) for i in range(n_tf)]
    tail_bg = [wd_rows(a, b - a) for a, b in zip((e0 + 8 * n_tf,) + tail_k[:-1], tail_k)]
    tail_sem = [sem.at[NPOS % _NS]] + [sem.at[_NS + t] for t in range(len(_TAIL_K))]
    tail_issue = [([(tail_bg[k], tail_sem[k], _BG)] if k < len(tail_bg) else [])
                  + [(tail_fg[k], tail_sem[0], _FG)] for k in range(n_tf)]

    mr, qr = wm.shape[1] // 8, wq.shape[1] // 8
    s_bg = [[same(wm_hbm, wm, (slice(None), pl.ds(8 * r, 8), pl.ds(col, _WM_C)))
             for col in range(0, 6 * D, _WM_C)] for r in range(mr)]
    wm_done = len(s_bg) - 1
    for r in range(qr - 1):
        s_bg += _split([same(wq_hbm, wq, (slice(None), pl.ds(8 * r, 8), pl.ds(col, _WQ_C)))
                        for col in range(0, H * DH, _WQ_C)], 3)
    n_s = len(s_bg)
    rest = [same(wq_hbm, wq, (st, pl.ds(8 * (qr - 1), 8), pl.ds(col, _WQ_F)))
            for st in range(_WQ_S) for col in range(0, H * DH, _WQ_F)]
    s_fg = [[lambda s: cp(c_hbm, cbuf, s), lambda s: cp(x_hbm, xbuf, s)]] + [[]] * (LA - 1)
    slots = [0]
    for g in range(n_s - LA):
        slots.append(slots[-1] + len(s_bg[g]))
    for a, b in zip(slots[:-1], slots[1:]):
        s_fg.append(rest[(a * len(rest)) // slots[-1]:(b * len(rest)) // slots[-1]])
    off = (-n_s) % _NS

    def ssem(g):
        return sem.at[(g + off) % _NS]

    for g in range(LA):
        for trip in plan(len(s_bg[g]), s_bg[g], s_fg[g], ssem(g)):
            for f, ns, prio in trip:
                f(ns).start(priority=prio)

    def load_x():
        return jnp.broadcast_to(xbuf[...].astype(F32), (8, D))

    def project_q(m):
        w2 = wq[:, :, pl.ds(mul(m, 2 * DH, 128), 2 * DH)].reshape(D, 2 * DH)
        q2 = _dot(h_scr[...].astype(BF16), w2)
        q_scr[0] = q2[:, 0:DH]
        q_scr[1] = q2[:, DH:2 * DH]

    fg0 = pair_fg(0)
    for g in range(n_s):
        gn = g + LA
        nbg, nfg = (s_bg[gn], s_fg[gn]) if gn < n_s else (kv_group(0, gn - n_s), fg0[gn - n_s])
        run_group(s_bg[g], s_fg[g], ssem(g), plan(len(s_bg[g]), nbg, nfg, ssem(gn)))
        k = g - wm_done
        if 0 <= k < 6:
            c = cbuf[...].astype(F32)
            sc = c * (1.0 / (1.0 + jnp.exp(-c)))
            sc8 = jnp.broadcast_to(sc, (8, D)).astype(BF16)
            wk = wm[:, :, k * D:(k + 1) * D].reshape(D, D)
            mod_scr[:, k * D:(k + 1) * D] = _rbf(_dot(sc8, wk))
        elif k == 6:
            sa, ca = mod_scr[:, 0:D], mod_scr[:, D:2 * D]
            h_scr[...] = _rbf(_rbf(_layernorm_rows(load_x())) * _rbf(1.0 + ca)) + sa
    project_q(0)

    def softmax():
        s = p_scr[...]
        e = jnp.exp(s - jnp.max(s, axis=-1, keepdims=True))
        l = jnp.sum(e, axis=-1, keepdims=True)
        p_scr[...] = _rbf(e * (1.0 / l))

    def pair_body(m, attn8, last):
        fg = pair_fg(m)
        fg_next = None if last else pair_fg(m + 1)
        acc = None
        for g in range(NPOS):
            gn = g + LA
            if gn < NPOS:
                issue = plan(_TPG, kv_group(m, gn), fg[gn], sem.at[gn % _NS])
            elif not last:
                issue = plan(_TPG, kv_group(m + 1, gn - NPOS), fg_next[gn - NPOS], sem.at[gn % _NS])
            else:
                issue = tail_issue[(gn - NPOS) * _TPG:(gn - NPOS + 1) * _TPG]
            mid = None
            if g % 8 == _NG:
                mid = softmax
            elif g == 8 + _NG + 1 and not last:
                mid = functools.partial(project_q, m + 1)
            run_group(kv_group(m, g), fg[g], sem.at[g % _NS], issue, mid)

            hh, j = g // 8, g % _NG
            if (g % 8) < _NG:
                s = _dot(q_scr[hh].astype(BF16), kbuf[j])
                p_scr[:, j * GW:(j + 1) * GW] = _rbf(_rbf(s) * scale)
                acc = jnp.zeros((DH // 8, 8, 128), F32)
            else:
                for t in range(GW // 256):
                    vt = vbuf[j, :, t * 256:(t + 1) * 256].astype(F32)
                    pj = p_scr[:, j * GW + t * 256:j * GW + (t + 1) * 256]
                    prod = vt.reshape(DH // 8, 8, 256) * pj[None]
                    acc = acc + prod[:, :, 0:128] + prod[:, :, 128:256]
                if j == _NG - 1:
                    o = _rbf(jnp.sum(acc, axis=-1, keepdims=True))
                    woh = wo[hh].astype(F32).reshape(DH // 8, 8, D)
                    attn8 = attn8 + jnp.sum(woh * o, axis=0)
        return attn8

    attn8 = lax.fori_loop(0, NP - 1, lambda m, a: pair_body(m, a, False),
                          jnp.zeros((8, D), F32))
    attn8 = pair_body(NP - 1, attn8, True)
    attn = _rbf(jnp.sum(attn8, axis=0, keepdims=True))

    ga, sb, cb, gb = [mod_scr[:, k * D:(k + 1) * D] for k in range(2, 6)]
    x1 = _rbf(load_x() + _rbf(ga * attn))
    h2 = (_rbf(_rbf(_layernorm_rows(x1)) * _rbf(1.0 + cb)) + sb).astype(BF16)
    g_ = _rbf(_dot(h2, wg[...]))
    u_ = _rbf(_dot(h2, wu[...]))
    gu = (g_ * u_).astype(BF16)
    hc0 = FF - _HC
    for f in tail_fg:
        f(tail_sem[0]).wait()
    n_t = len(tail_bg)
    for t in range(n_t):
        tail_bg[t](tail_sem[t]).wait()
        r0, r1 = (0 if t == 0 else tail_k[t - 1]), tail_k[t]
        if t == 0:
            hc_scr[...] = jnp.broadcast_to(gu[0:1, hc0:FF].astype(F32), (128, _HC)).T
        if t < n_t - _N_VPU:
            y = _dot(gu[:, r0:r1], wd[r0:r1, :])
            h_scr[...] = y if t == 0 else y + h_scr[...]
        else:
            n = (r1 - r0) // 8
            hc = hc_scr[r0 - hc0:r1 - hc0, :].reshape(n, 8, 128)
            hc = jnp.concatenate([hc] * (D // 128), axis=-1)
            z = jnp.sum(wd[r0:r1, :].astype(F32).reshape(n, 8, D) * hc, axis=0)
            if t > n_t - _N_VPU:
                z = z + z_scr[...]
            if t < n_t - 1:
                z_scr[...] = z
    y = h_scr[...] + jnp.sum(z, axis=0, keepdims=True)
    x2 = x1 + _rbf(gb * _rbf(y))
    out_ref[...] = x2[0:1, :].astype(out_ref.dtype)


def _compiler_params():
    opts = dict(vmem_limit_bytes=64 * 1024 * 1024, disable_semaphore_checks=True)
    known = {f.name for f in dataclasses.fields(pltpu.CompilerParams)}
    return pltpu.CompilerParams(**{k: v for k, v in opts.items() if k in known})


@jax.jit
def pallas_adaLN_cond__sliding_block_cached__glu_gated_bilinear__decode_kernel(
    A_x: jax.Array,
    A_k_cache: jax.Array,
    A_v_cache: jax.Array,
    A_wq: jax.Array,
    A_wo: jax.Array,
    B_x: jax.Array,
    B_w_gate: jax.Array,
    B_w_up: jax.Array,
    B_w_down: jax.Array,
    c: jax.Array,
    w_mod: jax.Array,
):
    B, SQ, D = A_x.shape
    _, HKV, SK, DH = A_k_cache.shape
    W = min(4096, max(256, SK // 4))
    FF = B_w_gate.shape[1]
    assert B == 1 and SQ == 1 and HKV == _HQ and DH == _DH
    assert (D, FF, W) == (640, 1536, _NG * _TPG * _CW)

    kt = jnp.swapaxes(A_k_cache, 2, 3).reshape(HKV * DH, SK)
    vt = jnp.swapaxes(A_v_cache, 2, 3).reshape(HKV * DH, SK)
    x2d = A_x.reshape(1, D)
    wq3 = A_wq.reshape(_WQ_S, D // _WQ_S, HKV * DH)
    wm3 = w_mod.reshape(_WM_S, D // _WM_S, 6 * D)

    any_spec = pl.BlockSpec(memory_space=pl.ANY)
    out = pl.pallas_call(
        functools.partial(_kernel, D=D, FF=FF, SK=SK, W=W),
        out_shape=jax.ShapeDtypeStruct((1, D), A_x.dtype),
        in_specs=[any_spec] * 10,
        out_specs=pl.BlockSpec(memory_space=pltpu.VMEM),
        scratch_shapes=[
            pltpu.VMEM((1, D), BF16),
            pltpu.VMEM((1, D), BF16),
            pltpu.VMEM((_NG, DH, _TPG * _CW), BF16),
            pltpu.VMEM((_NG, DH, _TPG * _CW), BF16),
            pltpu.VMEM(wq3.shape, BF16),
            pltpu.VMEM((2, DH, D), BF16),
            pltpu.VMEM(B_w_gate.shape, BF16),
            pltpu.VMEM(B_w_up.shape, BF16),
            pltpu.VMEM(B_w_down.shape, BF16),
            pltpu.VMEM(wm3.shape, BF16),
            pltpu.VMEM((2, 8, DH), F32),
            pltpu.VMEM((8, D), F32),
            pltpu.VMEM((8, 6 * D), F32),
            pltpu.VMEM((8, W), F32),
            pltpu.VMEM((_HC, 128), F32),
            pltpu.VMEM((8, D), F32),
            pltpu.SemaphoreType.DMA((_NS + len(_TAIL_K),)),
        ],
        compiler_params=_compiler_params(),
    )(x2d, c, kt, vt, wq3, A_wo, B_w_gate, B_w_up, B_w_down, wm3)
    return out.reshape(B, SQ, D)
```
